```python
import jax
import jax.numpy as jnp

def _softmax(x, axis=-1):
    return jax.nn.softmax(x, axis=axis)
def _gelu(x):
    return jax.nn.gelu(x, approximate=True)
def _silu(x):
    return jax.nn.silu(x)
def _sigmoid(x):
    return jax.nn.sigmoid(x)
def _layernorm(x, axis=-1, eps=1e-5):
    m = jnp.mean(x, axis=axis, keepdims=True)
    v = jnp.var(x, axis=axis, keepdims=True)
    return (x - m) / jnp.sqrt(v + eps)
def _scatter_add(tgt, idx, src, axis=0):
    return tgt.at[idx].add(src)
def _segment_sum(src, seg, n):
    return jax.ops.segment_sum(src, seg, n)
class _Rng:
    def __init__(self, key):
        self._k = key
    def _next(self):
        self._k, sub = jax.random.split(self._k)
        return sub
    def normal(self, shape):
        return jax.random.normal(self._next(), shape, dtype=jnp.bfloat16)
    def randint(self, lo, hi, shape):
        return jax.random.randint(self._next(), shape, lo, hi, dtype=jnp.int32)
    def uniform(self, shape, lo=0.0, hi=1.0):
        return jax.random.uniform(self._next(), shape, jnp.bfloat16, lo, hi)
    def permutation(self, n):
        return jax.random.permutation(self._next(), n)


kernel_name = 'recurrent_scan__ssm_conv_h3__mixer_token_mlp__prompt'

def setup_inputs():
    _rng = _Rng(jax.random.key(int.from_bytes(__import__("os").urandom(4), "little")))
    _w = (lambda a: (lambda t: t.astype(jnp.bfloat16) if jnp.issubdtype(t.dtype, jnp.floating) else t)(jnp.asarray(a)))
    def _A_setup():
        B, S, D = 1, 2048, 576
        ks = 4
        return {
            "q": _w((lambda *s: _rng.normal(s) * 0.05)(B, S, D)),
            "k": _w((lambda *s: _rng.normal(s) * 0.05)(B, S, D)),
            "v": _w((lambda *s: _rng.normal(s) * 0.05)(B, S, D)),
            "shift_k": _w((lambda *s: _rng.normal(s) * 0.05)(D, ks) * 0.5),
            "ssm_k": _w((lambda *s: _rng.normal(s) * 0.05)(D, S) * (1.0 / S ** 0.5)),
            "ssm_D": _w((lambda *s: _rng.normal(s) * 0.05)(D)),
        }
    _A_in = _A_setup()

    def _B_setup():
        B, S, D, F = 1, 2048, 576, 4608
        return {
            "x": _w((lambda *s: _rng.normal(s) * 0.05)(B, S, D)),
            "w1": _w((lambda *s: _rng.normal(s) * 0.05)(S, F) * (S ** -0.5)),
            "b1": _w((lambda *s: _rng.normal(s) * 0.05)(F) * 0.02),
            "w2": _w((lambda *s: _rng.normal(s) * 0.05)(F, S) * (F ** -0.5)),
            "b2": _w((lambda *s: _rng.normal(s) * 0.05)(S) * 0.02),
        }
    _B_in = _B_setup()

    return {
        "A_q": _A_in["q"],
        "A_k": _A_in["k"],
        "A_v": _A_in["v"],
        "A_shift_k": _A_in["shift_k"],
        "A_ssm_k": _A_in["ssm_k"],
        "A_ssm_D": _A_in["ssm_D"],
        "B_x": _B_in["x"],
        "B_w1": _B_in["w1"],
        "B_b1": _B_in["b1"],
        "B_w2": _B_in["w2"],
        "B_b2": _B_in["b2"],
    }

def reference(A_q, A_k, A_v, A_shift_k, A_ssm_k, A_ssm_D, B_x, B_w1, B_b1, B_w2, B_b2):
    def _A_ref(q, k, v, shift_k, ssm_k, ssm_D):
        B, S, D = q.shape
        ks = shift_k.shape[-1]
        k_pad = jnp.pad(k, ((0, 0), (ks - 1, 0), (0, 0)))
        k_shift = jnp.zeros_like(k)
        for t in range(ks):
            k_shift = k_shift + k_pad[:, t:t + S, :] * shift_k[:, ks - 1 - t][None, None, :]
        kv = k_shift * v
        L = 2 * S
        kv_pad = jnp.pad(kv, ((0, 0), (0, S), (0, 0)))
        kf_pad = jnp.pad(ssm_k, ((0, 0), (0, S)))
        kv_f = (lambda x, axes=(-2,-1): jnp.fft.rfft2(x.astype(jnp.float32), axes=axes))(kv_pad[:, None, :, :], axes=(1, 2))
        kf_f = (lambda x, axes=(-2,-1): jnp.fft.rfft2(x.astype(jnp.float32), axes=axes))(kf_pad[:, None, :], axes=(1, 2))
        kf_f = (lambda x, *d: x.transpose(*d))(kf_f, 1, 2, 0)
        y_f = kv_f * kf_f[None, :, :, :]
        y = (lambda x, s, axes=(-2,-1): jnp.fft.irfft2(x, s=s, axes=axes).astype(jnp.bfloat16))(y_f, (1, L), axes=(1, 2))[:, 0, :S, :]
        y = y + kv * ssm_D[None, None, :]
        return q * y

    def _B_ref(x, w1, b1, w2, b2):
        B, S, D = x.shape
        h = _layernorm(x, axis=-1)
        u = jnp.einsum("bsd,sf->bdf", h, w1) + b1
        u = _gelu(u)
        y = jnp.einsum("bdf,fs->bds", u, w2) + b2
        return (lambda x, *d: x.transpose(*d))(y, 0, 2, 1)

    x = A_q
    xn = _layernorm(x, axis=-1)
    s = _A_ref(xn, A_k, A_v, A_shift_k, A_ssm_k, A_ssm_D)
    g = _silu(_B_ref(xn, B_w1, B_b1, B_w2, B_b2))
    return x + s * g
```

```python
import jax, jax.numpy as jnp, numpy as np
from jax.experimental import pallas as pl
from jax.experimental.pallas import tpu as pltpu
import ml_dtypes

S, D, F = 2048, 576, 4608
BF = 512; BS = 256
N1 = F // BF; N2 = S // BS
GC = D // N1
C = 128
NC = S // C
EPS = 1e-5

def _dft_mats():
    t = np.arange(C)[:, None]; j = np.arange(C)[None, :]
    th = np.pi * (4 * j + 1) * t / (2 * C)
    fwd = np.concatenate([np.cos(th), np.sin(th)], axis=1)
    inv = fwd.T / C
    return fwd.astype(ml_dtypes.bfloat16), inv.astype(ml_dtypes.bfloat16)
_FWD, _INV = _dft_mats()

def gelu(u):
    c = 0.7978845608028654
    return 0.5 * u * (1 + jnp.tanh(c * (u + 0.044715 * u * u * u)))

def ln_prologue(x_ref, hT, xnT, sk_ref, dv_ref, par):
    x = x_ref[...].astype(jnp.float32)
    m = jnp.sum(x, axis=0, keepdims=True) * (1.0 / D)
    xc = x - m
    var = jnp.sum(xc * xc, axis=0, keepdims=True) * (1.0 / D)
    r1 = jax.lax.rsqrt(var + EPS)
    r2 = jax.lax.rsqrt(var * r1 * r1 + EPS)
    xnT[...] = (xc * r1).astype(jnp.bfloat16)
    hT[...] = (xc * (r1 * r2)).astype(jnp.bfloat16)

def par_prologue(sk_ref, dv_ref, par):
    rows = jnp.concatenate([sk_ref[...].astype(jnp.float32), dv_ref[...].astype(jnp.float32),
                            jnp.zeros((3, D), jnp.float32)], axis=0)
    colT = rows.T
    for j in range(5):
        par[:, j * 128:(j + 1) * 128] = jnp.broadcast_to(colT[:, j:j + 1], (D, 128))

def stack(a):
    return jnp.concatenate([a[:, c * C:(c + 1) * C] for c in range(NC)], axis=0)

def conv_group(g, k_ref, v_ref, kk_ref, xnT, par, fwd_ref, inv_ref, sT):
    r0 = pl.multiple_of(g * GC, GC)
    kf = k_ref[...].astype(jnp.float32)
    lane = jax.lax.broadcasted_iota(jnp.int32, (GC, 128), 1)
    def tap(j):
        return par[pl.ds(r0, GC), j * 128:(j + 1) * 128]
    acc = None
    for j in range(4):
        if j == 0:
            kj = kf
        else:
            rj = pltpu.roll(kf, j, axis=1)
            kj = jnp.concatenate([jnp.where(lane >= j, rj[:, :128], 0.0), rj[:, 128:]], axis=1)
        tj = tap(j)
        tj = jnp.concatenate([tj] * NC, axis=1)
        acc = kj * tj if acc is None else acc + kj * tj
    kv = acc * v_ref[...].astype(jnp.float32)
    fwd = fwd_ref[...]
    X = jnp.dot(stack(kv.astype(jnp.bfloat16)), fwd, preferred_element_type=jnp.float32)
    K = jnp.dot(stack(kk_ref[...]), fwd, preferred_element_type=jnp.float32)
    zre = [[None] * (GC // 8) for _ in range(NC)]
    zim = [[None] * (GC // 8) for _ in range(NC)]
    for r in range(GC // 8):
        def t(A, i, part):
            return A[i * GC + r * 8:i * GC + r * 8 + 8, part * C:(part + 1) * C]
        a = [t(X, i, 0) for i in range(NC)]
        b = [t(X, i, 1) for i in range(NC)]
        s = [a[i] + b[i] for i in range(NC)]
        kre = [t(K, i, 0) for i in range(NC)]
        kim = [t(K, i, 1) for i in range(NC)]
        c = [kre[0]] + [kre[d] + kim[d - 1] for d in range(1, NC)]
        dd = [kim[0]] + [kim[d] - kre[d - 1] for d in range(1, NC)]
        e = [dd[d] - c[d] for d in range(NC)]
        f = [c[d] + dd[d] for d in range(NC)]
        for m in range(NC):
            k1 = k2 = k3 = None
            for i in range(m + 1):
                p1 = c[m - i] * s[i]; p2 = e[m - i] * a[i]; p3 = f[m - i] * b[i]
                k1 = p1 if k1 is None else k1 + p1
                k2 = p2 if k2 is None else k2 + p2
                k3 = p3 if k3 is None else k3 + p3
            zre[m][r] = k1 - k3
            zim[m][r] = k1 + k2
    Z = jnp.concatenate([jnp.concatenate([jnp.concatenate(zre[m], axis=0), jnp.concatenate(zim[m], axis=0)], axis=1)
                         for m in range(NC)], axis=0)
    Y = jnp.dot(Z.astype(jnp.bfloat16), inv_ref[...], preferred_element_type=jnp.float32)
    y = jnp.concatenate([Y[m * GC:(m + 1) * GC, :] for m in range(NC)], axis=1)
    dcol = tap(4)
    dcol = jnp.concatenate([dcol] * NC, axis=1)
    sv = xnT[pl.ds(r0, GC), :].astype(jnp.float32) * (y + kv * dcol)
    sT[pl.ds(r0, GC), :] = sv.astype(jnp.bfloat16)

def mm1(i, hT, w1_ref, b1_ref, U):
    u = jnp.dot(hT[...], w1_ref[...], preferred_element_type=jnp.float32) + b1_ref[...].astype(jnp.float32)
    U[:, pl.ds(pl.multiple_of(i * BF, BF), BF)] = gelu(u).astype(jnp.bfloat16)

def kern(x_ref, k_ref, v_ref, kk_ref, sk_ref, dv_ref, w1_ref, b1_ref, w2_ref, b2_ref, fwd_ref, inv_ref,
         o_ref, hT, xnT, sT, U, par):
    i = pl.program_id(0)

    @pl.when(i == 0)
    def _():
        par_prologue(sk_ref, dv_ref, par)
        ln_prologue(x_ref, hT, xnT, sk_ref, dv_ref, par)

    @pl.when(i < N1)
    def _():
        mm1(i, hT, w1_ref, b1_ref, U)
        conv_group(i, k_ref, v_ref, kk_ref, xnT, par, fwd_ref, inv_ref, sT)

    @pl.when(i >= N1)
    def _():
        j = i - N1
        c0 = pl.multiple_of(j * BS, BS)
        y = jnp.dot(U[...], w2_ref[...], preferred_element_type=jnp.float32) + b2_ref[...].astype(jnp.float32)
        g = y * jax.nn.sigmoid(y)
        o_ref[...] = (x_ref[:, pl.ds(c0, BS)].astype(jnp.float32)
                      + sT[:, pl.ds(c0, BS)].astype(jnp.float32) * g).astype(jnp.bfloat16)

@jax.jit
def pallas_recurrent_scan__ssm_conv_h3__mixer_token_mlp__prompt_kernel(A_q, A_k, A_v, A_shift_k, A_ssm_k, A_ssm_D, B_x, B_w1, B_b1, B_w2, B_b2):
    xT = A_q.reshape(S, D).T
    kT = A_k.reshape(S, D).T
    vT = A_v.reshape(S, D).T
    p1 = lambda i: (jnp.minimum(i, N1 - 1), 0)
    c1 = lambda i: (0, jnp.minimum(i, N1 - 1))
    c2 = lambda i: (0, jnp.maximum(i - N1, 0))
    z = lambda i: (0, 0)
    outT = pl.pallas_call(kern,
        grid=(N1 + N2,),
        in_specs=[pl.BlockSpec((D, S), z),
                  pl.BlockSpec((GC, S), p1), pl.BlockSpec((GC, S), p1), pl.BlockSpec((GC, S), p1),
                  pl.BlockSpec((4, D), z), pl.BlockSpec((1, D), z),
                  pl.BlockSpec((S, BF), c1), pl.BlockSpec((1, BF), c1),
                  pl.BlockSpec((F, BS), c2), pl.BlockSpec((1, BS), c2),
                  pl.BlockSpec((C, 2 * C), z), pl.BlockSpec((2 * C, C), z)],
        out_specs=pl.BlockSpec((D, BS), c2),
        out_shape=jax.ShapeDtypeStruct((D, S), jnp.bfloat16),
        scratch_shapes=[pltpu.VMEM((D, S), jnp.bfloat16), pltpu.VMEM((D, S), jnp.bfloat16),
                        pltpu.VMEM((D, S), jnp.bfloat16), pltpu.VMEM((D, F), jnp.bfloat16),
                        pltpu.VMEM((D, 5 * 128), jnp.float32)],
        compiler_params=pltpu.CompilerParams(dimension_semantics=("arbitrary",), vmem_limit_bytes=100 << 20),
    )(xT, kT, vT, A_ssm_k, A_shift_k.T, A_ssm_D.reshape(1, D), B_w1, B_b1.reshape(1, F), B_w2, B_b2.reshape(1, S),
      jnp.asarray(_FWD), jnp.asarray(_INV))
    return outT.T.reshape(1, S, D)
```

```python
import jax, jax.numpy as jnp, numpy as np
from jax.experimental import pallas as pl
from jax.experimental.pallas import tpu as pltpu
import ml_dtypes

S, D, F = 2048, 576, 4608
BF = 512; BS = 256
N1 = F // BF; N2 = S // BS
GC = D // N1
C = 128
NC = S // C
EPS = 1e-5

def _dft_mats():
    t = np.arange(C)[:, None]; j = np.arange(C)[None, :]
    th = np.pi * (4 * j + 1) * t / (2 * C)
    fwd = np.concatenate([np.cos(th), np.sin(th)], axis=1)
    inv = fwd.T / C
    return fwd.astype(ml_dtypes.bfloat16), inv.astype(ml_dtypes.bfloat16)
_FWD, _INV = _dft_mats()

def pk(a): return pltpu.bitcast(a, jnp.uint32)
def upk(a): return pltpu.bitcast(a, jnp.bfloat16)

def gelu(u):
    c = 0.7978845608028654
    return 0.5 * u * (1 + jnp.tanh(c * (u + 0.044715 * u * u * u)))

def ln_prologue(x_ref, hT, xnT):
    x = x_ref[...].astype(jnp.float32)
    m = jnp.sum(x, axis=0, keepdims=True) * (1.0 / D)
    xc = x - m
    var = jnp.sum(xc * xc, axis=0, keepdims=True) * (1.0 / D)
    r1 = jax.lax.rsqrt(var + EPS)
    r2 = jax.lax.rsqrt(var * r1 * r1 + EPS)
    xnT[...] = pk((xc * r1).astype(jnp.bfloat16))
    hT[...] = pk((xc * (r1 * r2)).astype(jnp.bfloat16))

def par_prologue(sk_ref, dv_ref, par):
    rows = jnp.concatenate([sk_ref[...].astype(jnp.float32), dv_ref[...].astype(jnp.float32).reshape(1, D),
                            jnp.zeros((3, D), jnp.float32)], axis=0)
    colT = rows.T
    for j in range(5):
        par[:, j * 128:(j + 1) * 128] = jnp.broadcast_to(colT[:, j:j + 1], (D, 128))

def stack(a):
    return jnp.concatenate([a[:, c * C:(c + 1) * C] for c in range(NC)], axis=0)

OPAQUE = 1
def conv_segments(g, k_ref, v_ref, kk_ref, xnT, par, fwd_ref, inv_ref, sT, pb):
    st = {}
    r0 = pl.multiple_of(g * GC, GC)
    def tap(j):
        return par[pl.ds(r0, GC), j * 128:(j + 1) * 128]
    def segA():
        kf = k_ref[...].astype(jnp.float32)
        lane = jax.lax.broadcasted_iota(jnp.int32, (GC, 128), 1)
        acc = None
        for j in range(4):
            if j == 0:
                kj = kf
            else:
                rj = pltpu.roll(kf, j, axis=1)
                kj = jnp.concatenate([jnp.where(lane >= j, rj[:, :128], 0.0), rj[:, 128:]], axis=1)
            tj = tap(j)
            tj = jnp.concatenate([tj] * NC, axis=1)
            acc = kj * tj if acc is None else acc + kj * tj
        kv = acc * v_ref[...].astype(jnp.float32)
        st['kv'] = kv
        st['X'] = jnp.dot(stack(kv.astype(jnp.bfloat16)), fwd_ref[...], preferred_element_type=jnp.float32)
    def segK():
        st['K'] = jnp.dot(stack(kk_ref[...]), fwd_ref[...], preferred_element_type=jnp.float32)
    NT = GC // 8
    names = ['a', 'b', 's', 'c', 'e', 'f', 'k1', 'zre', 'zim']
    off = {n: k * NC * NT for k, n in enumerate(names)}
    zs = [pl.program_id(0) >> 6, pl.program_id(0) >> 7]
    cnt = [0]
    def nz():
        cnt[0] += 1
        return zs[cnt[0] % 2] if OPAQUE else 0
    def slot(n, i, r): return off[n] + i * NT + r
    def segQ(r):
        X, K = st['X'], st['K']
        z = st.setdefault('zq', 0)
        def t(A, i, part):
            return A[i * GC + r * 8:i * GC + r * 8 + 8, part * C:(part + 1) * C]
        for i in range(NC):
            a = t(X, i, 0); b = t(X, i, 1)
            pb[slot('a', i, r)] = a; pb[slot('b', i, r)] = b; pb[slot('s', i, r)] = a + b
        for d in range(NC):
            kre = t(K, d, 0); kim = t(K, d, 1)
            if d == 0:
                c, dd = kre, kim
            else:
                c = kre + t(K, d - 1, 1); dd = kim - t(K, d - 1, 0)
            pb[slot('c', d, r)] = c; pb[slot('e', d, r)] = dd - c; pb[slot('f', d, r)] = c + dd
    def rconv(p, q):
        out = []
        for m0 in range(0, NC, MB):
            ms = list(range(m0, min(m0 + MB, NC)))
            k = {m: None for m in ms}
            for i in range(ms[-1] + 1):
                for m in ms:
                    if i > m: continue
                    pr = q[m - i] * p[i]
                    k[m] = pr if k[m] is None else k[m] + pr
            out += [k[m] for m in ms]
        return out
    def segP(r):
        z = nz()
        p = [pb[z + slot('s', i, r)] for i in range(NC)]; q = [pb[z + slot('c', i, r)] for i in range(NC)]
        k1 = rconv(p, q)
        for m in range(NC): pb[z + slot('k1', m, r)] = k1[m]
        z = nz()
        p = [pb[z + slot('b', i, r)] for i in range(NC)]; q = [pb[z + slot('f', i, r)] for i in range(NC)]
        k3 = rconv(p, q)
        for m in range(NC): pb[z + slot('zre', m, r)] = pb[z + slot('k1', m, r)] - k3[m]
        z = nz()
        p = [pb[z + slot('a', i, r)] for i in range(NC)]; q = [pb[z + slot('e', i, r)] for i in range(NC)]
        k2 = rconv(p, q)
        for m in range(NC): pb[z + slot('zim', m, r)] = pb[z + slot('k1', m, r)] + k2[m]
    def segI():
        z = nz()
        rows = []
        for m in range(NC):
            re = jnp.concatenate([pb[z + slot('zre', m, r)] for r in range(NT)], axis=0)
            im = jnp.concatenate([pb[z + slot('zim', m, r)] for r in range(NT)], axis=0)
            rows.append(jnp.concatenate([re, im], axis=1))
        Z = jnp.concatenate(rows, axis=0)
        Y = jnp.dot(Z.astype(jnp.bfloat16), inv_ref[...], preferred_element_type=jnp.float32)
        y = jnp.concatenate([Y[m * GC:(m + 1) * GC, :] for m in range(NC)], axis=1)
        dcol = tap(4)
        dcol = jnp.concatenate([dcol] * NC, axis=1)
        r0h = pl.multiple_of(g * (GC // 2), GC // 2)
        sv = upk(xnT[pl.ds(r0h, GC // 2), :]).astype(jnp.float32) * (y + st['kv'] * dcol)
        sT[pl.ds(r0h, GC // 2), :] = pk(sv.astype(jnp.bfloat16))
    return segA, segK, segQ, segP, segI

MB = 4
NP = 4
def mm1_piece(i, t, hT, w1_ref, b1_ref, U):
    W = BF // NP
    u = jnp.dot(upk(hT[...]), w1_ref[:, t * W:(t + 1) * W], preferred_element_type=jnp.float32) + b1_ref[:, pl.ds(pl.multiple_of(i * BF + t * W, W), W)]
    U[:, pl.ds(pl.multiple_of(i * BF + t * W, W), W)] = pk(gelu(u).astype(jnp.bfloat16))

ORDER = 'K M0 A Q0 Q1 Q2 Q3 Q4 Q5 Q6 Q7 P0 M1 P1 P2 P3 M2 P4 P5 P6 P7 I M3'.split()

def mm1(i, hT, w1_ref, b1_ref, U):
    u = jnp.dot(hT[...], w1_ref[...], preferred_element_type=jnp.float32) + b1_ref[...].astype(jnp.float32)
    U[:, pl.ds(pl.multiple_of(i * BF, BF), BF)] = gelu(u).astype(jnp.bfloat16)

def kern(x_hbm, k_hbm, v_hbm, kk_hbm, sk_ref, dv_ref, w1_hbm, b1_ref, w2_hbm, b2_ref, fwd_ref, inv_ref,
         o_ref, hT, xnT, sT, U, par, pb, xb, kb, vb, kkb, w1b, w2b, b1s, b2s, sems):
    i = pl.program_id(0)
    slot = i % 2
    SX, SW1, SK, SV, SKK, SW2 = 0, 1, 3, 5, 7, 9

    def x_copy(): return pltpu.make_async_copy(x_hbm, xb, sems.at[SX])
    def w1_copy(j, sl): return pltpu.make_async_copy(w1_hbm.at[:, pl.ds(pl.multiple_of(j * BF, BF), BF)], w1b.at[sl], sems.at[SW1 + sl])
    def grp_copies(j, sl):
        r = pl.ds(pl.multiple_of(j * GC, GC), GC)
        return [pltpu.make_async_copy(k_hbm.at[r, :], kb.at[sl], sems.at[SK + sl]),
                pltpu.make_async_copy(v_hbm.at[r, :], vb.at[sl], sems.at[SV + sl]),
                pltpu.make_async_copy(kk_hbm.at[r, :], kkb.at[sl], sems.at[SKK + sl])]
    def w2_copy(j, sl): return pltpu.make_async_copy(w2_hbm.at[:, pl.ds(pl.multiple_of(j * BS, BS), BS)], w2b.at[sl], sems.at[SW2 + sl])

    @pl.when(i == 0)
    def _():
      with jax.named_scope('start'):
        x_copy().start()
        w1_copy(0, 0).start()
        for c in grp_copies(0, 0): c.start()

    @pl.when(i + 1 < N1)
    def _():
        w1_copy(i + 1, 1 - slot).start()
        for c in grp_copies(i + 1, 1 - slot): c.start()

    @pl.when(i == W2START)
    def _():
        w2_copy(0, 0).start()

    @pl.when(jnp.logical_and(i >= N1, i + 1 < N1 + N2))
    def _():
        w2_copy(i - N1 + 1, 1 - (i - N1) % 2).start()

    @pl.when(i == 0)
    def _():
      with jax.named_scope('prologue'):
        par_prologue(sk_ref, dv_ref, par)
        b1s[...] = b1_ref[...].astype(jnp.float32).reshape(1, F)
        b2s[...] = b2_ref[...].astype(jnp.float32).reshape(1, S)
        x_copy().wait()
        ln_prologue(xb, hT, xnT)

    @pl.when(i < N1)
    def _():
      with jax.named_scope('ph1'):
        w1_copy(i, slot).wait()
        for c in grp_copies(i, slot): c.wait()
        w1_ref = w1b.at[slot]
        segA, segK, segQ, segP, segI = conv_segments(i, kb.at[slot], vb.at[slot], kkb.at[slot], xnT, par, fwd_ref, inv_ref, sT, pb)
        for o in ORDER:
            if o == 'A': segA()
            elif o == 'K': segK()
            elif o == 'I': segI()
            elif o[0] == 'Q': segQ(int(o[1:]))
            elif o[0] == 'P': segP(int(o[1:]))
            elif o[0] == 'M': mm1_piece(i, int(o[1:]), hT, w1_ref, b1s, U)

    @pl.when(i >= N1)
    def _():
      with jax.named_scope('ph2'):
        j = i - N1
        sl = j % 2
        w2_copy(j, sl).wait()
        c0 = pl.multiple_of(j * BS, BS)
        y = jnp.dot(upk(U[...]), w2b[sl], preferred_element_type=jnp.float32) + b2s[:, pl.ds(c0, BS)]
        g = y * jax.nn.sigmoid(y)
        o_ref[...] = (xb[:, pl.ds(c0, BS)].astype(jnp.float32)
                      + upk(sT[:, pl.ds(c0, BS)]).astype(jnp.float32) * g).astype(jnp.bfloat16)

W2START = 4

@jax.jit
def pallas_recurrent_scan__ssm_conv_h3__mixer_token_mlp__prompt_kernel(A_q, A_k, A_v, A_shift_k, A_ssm_k, A_ssm_D, B_x, B_w1, B_b1, B_w2, B_b2):
    xT = A_q.reshape(S, D).T
    kT = A_k.reshape(S, D).T
    vT = A_v.reshape(S, D).T
    c2 = lambda i: (0, jnp.maximum(i - N1, 0))
    z = lambda i: (0, 0)
    z1 = lambda i: (0,)
    anyspec = pl.BlockSpec(memory_space=pl.ANY)
    u32 = jnp.uint32; bf = jnp.bfloat16; f32 = jnp.float32
    outT = pl.pallas_call(kern,
        grid=(N1 + N2,),
        in_specs=[anyspec, anyspec, anyspec, anyspec,
                  pl.BlockSpec((4, D), z), pl.BlockSpec((D,), z1),
                  anyspec, pl.BlockSpec((F,), z1), anyspec, pl.BlockSpec((S,), z1),
                  pl.BlockSpec((C, 2 * C), z), pl.BlockSpec((2 * C, C), z)],
        out_specs=pl.BlockSpec((D, BS), c2),
        out_shape=jax.ShapeDtypeStruct((D, S), bf),
        scratch_shapes=[pltpu.VMEM((D // 2, S), u32), pltpu.VMEM((D // 2, S), u32),
                        pltpu.VMEM((D // 2, S), u32), pltpu.VMEM((D // 2, F), u32),
                        pltpu.VMEM((D, 5 * 128), f32), pltpu.VMEM((9 * NC * (GC // 8), 8, 128), f32),
                        pltpu.VMEM((D, S), bf), pltpu.VMEM((2, GC, S), bf), pltpu.VMEM((2, GC, S), bf), pltpu.VMEM((2, GC, S), bf),
                        pltpu.VMEM((2, S, BF), bf), pltpu.VMEM((2, F, BS), bf),
                        pltpu.VMEM((1, F), f32), pltpu.VMEM((1, S), f32),
                        pltpu.SemaphoreType.DMA((11,))],
        compiler_params=pltpu.CompilerParams(dimension_semantics=("arbitrary",), vmem_limit_bytes=100 << 20),
    )(xT, kT, vT, A_ssm_k, A_shift_k.T, A_ssm_D, B_w1, B_b1, B_w2, B_b2,
      jnp.asarray(_FWD), jnp.asarray(_INV))
    return outT.T.reshape(1, S, D)
```

```python
import jax, jax.numpy as jnp, numpy as np
from jax.experimental import pallas as pl
from jax.experimental.pallas import tpu as pltpu
import ml_dtypes

S, D, F = 2048, 576, 4608
N1 = 9; N2 = 8
BF = F // N1; BS = S // N2
GC = D // N1
NT = GC // 8
C = 128
NC = S // C
EPS = 1e-5
CH = 8; CW = S // CH
PRE = 5; LATE = 6
MB = 4

def _dft_mats():
    t = np.arange(C)[:, None]; j = np.arange(C)[None, :]
    th = np.pi * (4 * j + 1) * t / (2 * C)
    fwd = np.concatenate([np.cos(th), np.sin(th)], axis=1)
    inv = fwd.T / C
    return fwd.astype(ml_dtypes.bfloat16), inv.astype(ml_dtypes.bfloat16)
_FWD, _INV = _dft_mats()

def pk(a): return pltpu.bitcast(a, jnp.uint32)
def upk(a): return pltpu.bitcast(a, jnp.bfloat16)
f32 = jnp.float32; bf16 = jnp.bfloat16

def gelu(u):
    c = 0.7978845608028654
    hu = 0.5 * u
    return hu + hu * jnp.tanh(u * (c + (c * 0.044715) * (u * u)))

def silu(y):
    hy = 0.5 * y
    return hy + hy * jnp.tanh(hy)

def par_prologue(sk_ref, dv_ref, par):
    rows = jnp.concatenate([sk_ref[...].astype(f32), dv_ref[...].astype(f32).reshape(1, D),
                            jnp.zeros((3, D), f32)], axis=0)
    colT = rows.T
    for j in range(5):
        par[:, j * 128:(j + 1) * 128] = jnp.broadcast_to(colT[:, j:j + 1], (D, 128))

def stack(a):
    return jnp.concatenate([a[:, c * C:(c + 1) * C] for c in range(NC)], axis=0)

def ln_chunk(xb, hT, xnT, c):
    cs = slice(c * CW, (c + 1) * CW)
    x = xb[:, cs].astype(f32)
    m = jnp.sum(x, axis=0, keepdims=True) * (1.0 / D)
    xc = x - m
    var = jnp.sum(xc * xc, axis=0, keepdims=True) * (1.0 / D)
    r1 = jax.lax.rsqrt(var + EPS)
    r2 = jax.lax.rsqrt(var * r1 * r1 + EPS)
    xnT[:, cs] = pk((xc * r1).astype(bf16))
    h = (xc * (r1 * r2)).astype(bf16)
    hT[:, cs] = pk(h)
    return h

def conv_segments(g, k_ref, v_ref, kk_ref, xnT, par, fwd_ref, inv_ref, sT, pb):
    st = {}
    r0 = pl.multiple_of(g * GC, GC)
    def tap(j):
        t = par[pl.ds(r0, GC), j * 128:(j + 1) * 128]
        return jnp.concatenate([t] * NC, axis=1)
    def segA():
        kf = k_ref[...].astype(f32)
        lane = jax.lax.broadcasted_iota(jnp.int32, (GC, 128), 1)
        acc = None
        for j in range(4):
            if j == 0:
                kj = kf
            else:
                rj = pltpu.roll(kf, j, axis=1)
                kj = jnp.concatenate([jnp.where(lane >= j, rj[:, :128], 0.0), rj[:, 128:]], axis=1)
            acc = kj * tap(j) if acc is None else acc + kj * tap(j)
        kv = acc * v_ref[...].astype(f32)
        st['kv'] = kv
        st['X'] = jnp.dot(stack(kv.astype(bf16)), fwd_ref[...], preferred_element_type=f32)
    def segK():
        st['K'] = jnp.dot(stack(kk_ref[...]), fwd_ref[...], preferred_element_type=f32)
    names = ['a', 'b', 's', 'c', 'e', 'f', 'k1', 'zre', 'zim']
    off = {n: k * NC * NT for k, n in enumerate(names)}
    zs = [pl.program_id(0) >> 6, pl.program_id(0) >> 7]
    cnt = [0]
    def nz():
        cnt[0] += 1
        return zs[cnt[0] % 2]
    def slot(n, i, r): return off[n] + i * NT + r
    def segQ(r):
        X, K = st['X'], st['K']
        def t(A, i, part):
            return A[i * GC + r * 8:i * GC + r * 8 + 8, part * C:(part + 1) * C]
        for i in range(NC):
            a = t(X, i, 0); b = t(X, i, 1)
            pb[slot('a', i, r)] = a; pb[slot('b', i, r)] = b; pb[slot('s', i, r)] = a + b
        for d in range(NC):
            kre = t(K, d, 0); kim = t(K, d, 1)
            if d == 0:
                c, dd = kre, kim
            else:
                c = kre + t(K, d - 1, 1); dd = kim - t(K, d - 1, 0)
            pb[slot('c', d, r)] = c; pb[slot('e', d, r)] = dd - c; pb[slot('f', d, r)] = c + dd
    def rconv(p, q):
        out = []
        for m0 in range(0, NC, MB):
            ms = list(range(m0, min(m0 + MB, NC)))
            k = {m: None for m in ms}
            for i in range(ms[-1] + 1):
                for m in ms:
                    if i > m: continue
                    pr = q[m - i] * p[i]
                    k[m] = pr if k[m] is None else k[m] + pr
            out += [k[m] for m in ms]
        return out
    def segP(r):
        z = nz()
        p = [pb[z + slot('s', i, r)] for i in range(NC)]; q = [pb[z + slot('c', i, r)] for i in range(NC)]
        k1 = rconv(p, q)
        for m in range(NC): pb[z + slot('k1', m, r)] = k1[m]
        z = nz()
        p = [pb[z + slot('b', i, r)] for i in range(NC)]; q = [pb[z + slot('f', i, r)] for i in range(NC)]
        k3 = rconv(p, q)
        for m in range(NC): pb[z + slot('zre', m, r)] = pb[z + slot('k1', m, r)] - k3[m]
        z = nz()
        p = [pb[z + slot('a', i, r)] for i in range(NC)]; q = [pb[z + slot('e', i, r)] for i in range(NC)]
        k2 = rconv(p, q)
        for m in range(NC): pb[z + slot('zim', m, r)] = pb[z + slot('k1', m, r)] + k2[m]
    def segI():
        z = nz()
        rows = []
        for m in range(NC):
            re = jnp.concatenate([pb[z + slot('zre', m, r)] for r in range(NT)], axis=0)
            im = jnp.concatenate([pb[z + slot('zim', m, r)] for r in range(NT)], axis=0)
            rows.append(jnp.concatenate([re, im], axis=1))
        Z = jnp.concatenate(rows, axis=0)
        Y = jnp.dot(Z.astype(bf16), inv_ref[...], preferred_element_type=f32)
        y = jnp.concatenate([Y[m * GC:(m + 1) * GC, :] for m in range(NC)], axis=1)
        r0h = pl.multiple_of(g * (GC // 2), GC // 2)
        sv = upk(xnT[pl.ds(r0h, GC // 2), :]).astype(f32) * (y + st['kv'] * tap(4))
        sT[pl.ds(r0h, GC // 2), :] = pk(sv.astype(bf16))
    return segA, segK, segQ, segP, segI

def make_order(npieces):
    order = ['K', 'M0', 'A'] + ['Q%d' % r for r in range(NT)]
    mid = list(range(1, npieces - 1))
    ev = [((r + 0.5) / NT, 'P%d' % r) for r in range(NT)] + [((k + MOFF) / max(len(mid), 1), 'M%d' % t) for k, t in enumerate(mid)]
    order += [e[1] for e in sorted(ev)]
    order += ['I', 'M%d' % (npieces - 1)]
    return order
MOFF = 0.3

def mm1_piece(i, t, hT, w1_ref, b1s, U):
    cols = pl.ds(pl.multiple_of(i * BF + t * 128, 128), 128)
    u = jnp.dot(upk(hT[...]), w1_ref[:, t * 128:(t + 1) * 128], preferred_element_type=f32) + b1s[:, cols]
    U[:, cols] = pk(gelu(u).astype(bf16))

def epilogue(j, y, xb, sT, o_ref):
    c0 = pl.multiple_of(j * BS, BS)
    o_ref[...] = (xb[:, pl.ds(c0, BS)].astype(f32) + upk(sT[:, pl.ds(c0, BS)]).astype(f32) * silu(y)).astype(bf16)

def kern(x_hbm, k_hbm, v_hbm, kk_hbm, sk_ref, dv_ref, w1_hbm, b1_ref, w2_hbm, b2_ref, fwd_ref, inv_ref,
         o_ref, hT, xnT, sT, U, par, pb, xb, kb, vb, kkb, w1b, w2b, b1s, b2s, ybuf, sems):
    i = pl.program_id(0)
    slot = i % 2
    SW1, SK, SV, SKK, SW2, SX, SW10 = 0, 2, 4, 6, 8, 10, 10 + CH

    def x_copy(c): return pltpu.make_async_copy(x_hbm.at[:, c * CW:(c + 1) * CW], xb.at[:, c * CW:(c + 1) * CW], sems.at[SX + c])
    def w10_copy(c): return pltpu.make_async_copy(w1_hbm.at[c * CW:(c + 1) * CW, 0:BF], w1b.at[0, c * CW:(c + 1) * CW, :], sems.at[SW10 + c])
    def w1_copy(j, sl): return pltpu.make_async_copy(w1_hbm.at[:, pl.ds(pl.multiple_of(j * BF, 128), BF)], w1b.at[sl], sems.at[SW1 + sl])
    def grp_copies(j, sl):
        r = pl.ds(pl.multiple_of(j * GC, 16), GC)
        return [pltpu.make_async_copy(kk_hbm.at[r, :], kkb.at[sl], sems.at[SKK + sl]),
                pltpu.make_async_copy(k_hbm.at[r, :], kb.at[sl], sems.at[SK + sl]),
                pltpu.make_async_copy(v_hbm.at[r, :], vb.at[sl], sems.at[SV + sl])]
    def w2_copy(j, sl): return pltpu.make_async_copy(w2_hbm.at[:, pl.ds(pl.multiple_of(j * BS, BS), BS)], w2b.at[sl], sems.at[SW2 + sl])

    def run_order(order, g, gslot, mpiece):
        segA, segK, segQ, segP, segI = conv_segments(g, kb.at[gslot], vb.at[gslot], kkb.at[gslot], xnT, par, fwd_ref, inv_ref, sT, pb)
        for o in order:
            if o == 'A': segA()
            elif o == 'K': segK()
            elif o == 'I': segI()
            elif o[0] == 'Q': segQ(int(o[1:]))
            elif o[0] == 'P': segP(int(o[1:]))
            else: mpiece(int(o[1:]))

    def mm2_tile(j, sl):
        part = {}
        KH = F // 2
        c0 = pl.multiple_of(j * BS, BS)
        def mp(t):
            nt, kh = t // 2, t % 2
            part[t] = jnp.dot(upk(U[:, kh * KH:(kh + 1) * KH]), w2b[sl, kh * KH:(kh + 1) * KH, nt * 128:(nt + 1) * 128], preferred_element_type=f32)
            if kh == 1:
                ybuf[sl, :, nt * 128:(nt + 1) * 128] = part[t - 1] + part[t] + b2s[:, pl.ds(pl.multiple_of(c0 + nt * 128, 128), 128)]
        return mp

    @pl.when(i == 0)
    def _():
      with jax.named_scope('s0'):
        seq = [('x', 0)]
        for c in range(CH):
            if c + 1 < CH: seq.append(('x', c + 1))
            seq.append(('w', c))
        nissued = [0]
        def issue_upto(n):
            while nissued[0] < min(n, len(seq)):
                kind, c = seq[nissued[0]]
                (x_copy(c) if kind == 'x' else w10_copy(c)).start()
                nissued[0] += 1
        issue_upto(PRE)
        par_prologue(sk_ref, dv_ref, par)
        b1s[...] = b1_ref[...].astype(f32).reshape(1, F)
        b2s[...] = b2_ref[...].astype(f32).reshape(1, S)
        x_copy(0).wait()
        hs = {0: ln_chunk(xb, hT, xnT, 0)}
        acc = None
        for c in range(CH):
            if c + 1 < CH: x_copy(c + 1).wait()
            w10_copy(c).wait()
            issue_upto(PRE + 2 * (c + 1))
            if c == max(CH - 1 - LATE, 0):
                issue_upto(len(seq))
                cps = grp_copies(0, 1)
                cps[0].start()
                if N1 > 1: w1_copy(1, 1).start()
                cps[1].start(); cps[2].start()
            d = jnp.dot(hs[c], w1b[0, c * CW:(c + 1) * CW, :], preferred_element_type=f32)
            acc = d if acc is None else acc + d
            if c + 1 < CH: hs[c + 1] = ln_chunk(xb, hT, xnT, c + 1)
        U[:, 0:BF] = pk(gelu(acc + b1s[:, 0:BF]).astype(bf16))

    @pl.when(jnp.logical_and(i >= 1, i < N1 - 1))
    def _():
        w1_copy(i + 1, 1 - slot).start()
    @pl.when(i == N1 - 1)
    def _():
        w2_copy(0, 0).start()
    @pl.when(jnp.logical_and(i >= 1, i < N1))
    def _():
      with jax.named_scope('ph1'):
        for cp in grp_copies(i, 1 - slot): cp.start()
        w1_copy(i, slot).wait()
        for cp in grp_copies(i - 1, slot): cp.wait()
        run_order(make_order(BF // 128), i - 1, slot, lambda t: mm1_piece(i, t, hT, w1b.at[slot], b1s, U))

    @pl.when(i == N1)
    def _():
      with jax.named_scope('ph1b'):
        if N2 > 1: w2_copy(1, 1).start()
        w2_copy(0, 0).wait()
        for cp in grp_copies(N1 - 1, N1 % 2): cp.wait()
        run_order(make_order(2 * (BS // 128)), N1 - 1, N1 % 2, mm2_tile(0, 0))

    @pl.when(jnp.logical_and(i > N1, i < N1 + N2 - 1))
    def _():
        w2_copy(i - N1 + 1, (i - N1 + 1) % 2).start()
    @pl.when(jnp.logical_and(i > N1, i < N1 + N2))
    def _():
      with jax.named_scope('ph2'):
        j = i - N1
        sl = j % 2
        w2_copy(j, sl).wait()
        epilogue(j - 1, ybuf[1 - sl], xb, sT, o_ref)
        ybuf[sl] = jnp.dot(upk(U[...]), w2b[sl], preferred_element_type=f32) + b2s[:, pl.ds(pl.multiple_of(j * BS, BS), BS)]

    @pl.when(i == N1 + N2)
    def _():
      with jax.named_scope('fin'):
        epilogue(N2 - 1, ybuf[(N2 - 1) % 2], xb, sT, o_ref)

@jax.jit
def pallas_recurrent_scan__ssm_conv_h3__mixer_token_mlp__prompt_kernel(A_q, A_k, A_v, A_shift_k, A_ssm_k, A_ssm_D, B_x, B_w1, B_b1, B_w2, B_b2):
    xT = A_q.reshape(S, D).T
    kT = A_k.reshape(S, D).T
    vT = A_v.reshape(S, D).T
    c2 = lambda i: (0, jnp.clip(i - N1 - 1, 0, N2 - 1))
    z = lambda i: (0, 0)
    z1 = lambda i: (0,)
    anyspec = pl.BlockSpec(memory_space=pl.ANY)
    u32 = jnp.uint32; bf = jnp.bfloat16
    outT = pl.pallas_call(kern,
        grid=(N1 + N2 + 1,),
        in_specs=[anyspec, anyspec, anyspec, anyspec,
                  pl.BlockSpec((4, D), z), pl.BlockSpec((D,), z1),
                  anyspec, pl.BlockSpec((F,), z1), anyspec, pl.BlockSpec((S,), z1),
                  pl.BlockSpec((C, 2 * C), z), pl.BlockSpec((2 * C, C), z)],
        out_specs=pl.BlockSpec((D, BS), c2),
        out_shape=jax.ShapeDtypeStruct((D, S), bf),
        scratch_shapes=[pltpu.VMEM((D // 2, S), u32), pltpu.VMEM((D // 2, S), u32),
                        pltpu.VMEM((D // 2, S), u32), pltpu.VMEM((D // 2, F), u32),
                        pltpu.VMEM((D, 5 * 128), f32), pltpu.VMEM((9 * NC * NT, 8, 128), f32),
                        pltpu.VMEM((D, S), bf), pltpu.VMEM((2, GC, S), bf), pltpu.VMEM((2, GC, S), bf), pltpu.VMEM((2, GC, S), bf),
                        pltpu.VMEM((2, S, BF), bf), pltpu.VMEM((2, F, BS), bf),
                        pltpu.VMEM((1, F), f32), pltpu.VMEM((1, S), f32), pltpu.VMEM((2, D, BS), f32),
                        pltpu.SemaphoreType.DMA((10 + 2 * CH,))],
        compiler_params=pltpu.CompilerParams(dimension_semantics=("arbitrary",), vmem_limit_bytes=110 << 20),
    )(xT, kT, vT, A_ssm_k, A_shift_k.T, A_ssm_D, B_w1, B_b1, B_w2, B_b2,
      jnp.asarray(_FWD), jnp.asarray(_INV))
    return outT.T.reshape(1, S, D)
```

```python
import jax, jax.numpy as jnp, numpy as np
from jax.experimental import pallas as pl
from jax.experimental.pallas import tpu as pltpu
import ml_dtypes

S, D, F = 2048, 576, 4608
N1 = 6; N2 = 8
BF = F // N1; BS = S // N2
GC = D // N1
NT = GC // 8
C = 128
NC = S // C
EPS = 1e-5
CH = 8; CW = S // CH
PRE = 7; LATE = 6
MB = 4
PZ = 2
PRE0 = 0
PARPOS = 7
YB = 1
MERGE = 0
P2 = 1
DBC = 1

def _dft_mats():
    t = np.arange(C)[:, None]; j = np.arange(C)[None, :]
    th = np.pi * (4 * j + 1) * t / (2 * C)
    fwd = np.concatenate([np.cos(th), np.sin(th)], axis=1)
    inv = fwd.T / C
    return fwd.astype(ml_dtypes.bfloat16), inv.astype(ml_dtypes.bfloat16)
_FWD, _INV = _dft_mats()

def pk(a): return pltpu.bitcast(a, jnp.uint32)
def upk(a): return pltpu.bitcast(a, jnp.bfloat16)
f32 = jnp.float32; bf16 = jnp.bfloat16

def gelu(u):
    c = 0.7978845608028654
    hu = 0.5 * u
    return hu + hu * jnp.tanh(u * (c + (c * 0.044715) * (u * u)))

def silu(y):
    hy = 0.5 * y
    return hy + hy * jnp.tanh(hy)

def par_prologue(sk_ref, dv_ref, par):
    rows = jnp.concatenate([sk_ref[...].astype(f32), dv_ref[...].astype(f32).reshape(1, D),
                            jnp.zeros((3, D), f32)], axis=0)
    colT = rows.T
    for j in range(5):
        par[:, j * 128:(j + 1) * 128] = jnp.broadcast_to(colT[:, j:j + 1], (D, 128))

def stack(a):
    return jnp.concatenate([a[:, c * C:(c + 1) * C] for c in range(NC)], axis=0)

def ln_chunk(xb, hT, xnT, c):
    cs = slice(c * CW, (c + 1) * CW)
    x = xb[:, cs].astype(f32)
    m = jnp.sum(x, axis=0, keepdims=True) * (1.0 / D)
    xc = x - m
    var = jnp.sum(xc * xc, axis=0, keepdims=True) * (1.0 / D)
    r1 = jax.lax.rsqrt(var + EPS)
    r2 = jax.lax.rsqrt(var * r1 * r1 + EPS)
    xnT[:, cs] = pk((xc * r1).astype(bf16))
    h = (xc * (r1 * r2)).astype(bf16)
    hT[:, cs] = pk(h)
    return h

def conv_segments(g, k_ref, v_ref, kk_ref, xnT, par, fwd_ref, inv_ref, sT, pb):
    st = {}
    r0 = pl.multiple_of(g * GC, GC)
    def tap(j):
        t = par[pl.ds(r0, GC), j * 128:(j + 1) * 128]
        return jnp.concatenate([t] * NC, axis=1)
    def segA():
        kf = k_ref[...].astype(f32)
        lane = jax.lax.broadcasted_iota(jnp.int32, (GC, 128), 1)
        acc = None
        for j in range(4):
            if j == 0:
                kj = kf
            else:
                rj = pltpu.roll(kf, j, axis=1)
                kj = jnp.concatenate([jnp.where(lane >= j, rj[:, :128], 0.0), rj[:, 128:]], axis=1)
            acc = kj * tap(j) if acc is None else acc + kj * tap(j)
        kv = acc * v_ref[...].astype(f32)
        st['kv'] = kv
        if MERGE:
            XK = jnp.dot(jnp.concatenate([stack(kk_ref[...]), stack(kv.astype(bf16))], axis=0), fwd_ref[...], preferred_element_type=f32)
            st['K'] = XK[:NC * GC]; st['X'] = XK[NC * GC:]
        else:
            st['X'] = jnp.dot(stack(kv.astype(bf16)), fwd_ref[...], preferred_element_type=f32)
    def segK():
        if not MERGE:
            st['K'] = jnp.dot(stack(kk_ref[...]), fwd_ref[...], preferred_element_type=f32)
    names = ['a', 'b', 's', 'c', 'e', 'f', 'k1', 'zre', 'zim']
    off = {n: k * NC * NT for k, n in enumerate(names)}
    zs = [pl.program_id(0) >> 6, pl.program_id(0) >> 7]
    cnt = [0]
    def nz():
        cnt[0] += 1
        return zs[cnt[0] % 2]
    def slot(n, i, r): return off[n] + i * NT + r
    def segQ(r):
        X, K = st['X'], st['K']
        def t(A, i, part):
            return A[i * GC + r * 8:i * GC + r * 8 + 8, part * C:(part + 1) * C]
        for i in range(NC):
            a = t(X, i, 0); b = t(X, i, 1)
            pb[slot('a', i, r)] = a; pb[slot('b', i, r)] = b; pb[slot('s', i, r)] = a + b
        for d in range(NC):
            kre = t(K, d, 0); kim = t(K, d, 1)
            if d == 0:
                c, dd = kre, kim
            else:
                c = kre + t(K, d - 1, 1); dd = kim - t(K, d - 1, 0)
            pb[slot('c', d, r)] = c; pb[slot('e', d, r)] = dd - c; pb[slot('f', d, r)] = c + dd
    def rconv(p, q):
        out = []
        for m0 in range(0, NC, MB):
            ms = list(range(m0, min(m0 + MB, NC)))
            k = {m: None for m in ms}
            for i in range(ms[-1] + 1):
                for m in ms:
                    if i > m: continue
                    pr = q[m - i] * p[i]
                    k[m] = pr if k[m] is None else k[m] + pr
            out += [k[m] for m in ms]
        return out
    def segP(r):
        z = nz()
        p = [pb[z + slot('s', i, r)] for i in range(NC)]; q = [pb[z + slot('c', i, r)] for i in range(NC)]
        k1 = rconv(p, q)
        if PZ == 1:
            for m in range(NC): pb[z + slot('k1', m, r)] = k1[m]
            z = nz()
        p = [pb[z + slot('b', i, r)] for i in range(NC)]; q = [pb[z + slot('f', i, r)] for i in range(NC)]
        k3 = rconv(p, q)
        for m in range(NC): pb[z + slot('zre', m, r)] = (pb[z + slot('k1', m, r)] if PZ == 1 else k1[m]) - k3[m]
        if PZ >= 1: z = nz()
        p = [pb[z + slot('a', i, r)] for i in range(NC)]; q = [pb[z + slot('e', i, r)] for i in range(NC)]
        k2 = rconv(p, q)
        for m in range(NC): pb[z + slot('zim', m, r)] = (pb[z + slot('k1', m, r)] if PZ == 1 else k1[m]) + k2[m]
    def segI():
        z = nz()
        rows = []
        for m in range(NC):
            re = jnp.concatenate([pb[z + slot('zre', m, r)] for r in range(NT)], axis=0)
            im = jnp.concatenate([pb[z + slot('zim', m, r)] for r in range(NT)], axis=0)
            rows.append(jnp.concatenate([re, im], axis=1))
        Z = jnp.concatenate(rows, axis=0)
        Y = jnp.dot(Z.astype(bf16), inv_ref[...], preferred_element_type=f32)
        y = jnp.concatenate([Y[m * GC:(m + 1) * GC, :] for m in range(NC)], axis=1)
        r0h = pl.multiple_of(g * (GC // 2), GC // 2)
        sv = upk(xnT[pl.ds(r0h, GC // 2), :]).astype(f32) * (y + st['kv'] * tap(4))
        sT[pl.ds(r0h, GC // 2), :] = pk(sv.astype(bf16))
    return segA, segK, segQ, segP, segI

def make_order(npieces):
    order = ['K', 'M0', 'A'] + ['Q%d' % r for r in range(NT)]
    mid = list(range(1, npieces - 1))
    ev = [((r + 0.5) / NT, 'P%d' % r) for r in range(NT)] + [((k + MOFF) / max(len(mid), 1), 'M%d' % t) for k, t in enumerate(mid)]
    order += [e[1] for e in sorted(ev)]
    order += ['I', 'M%d' % (npieces - 1)]
    ov = ''
    if ov:
        order = []
        for tok in ov.split():
            order += ['Q%d' % r for r in range(NT)] if tok == 'Q' else [tok]
    return order
MOFF = 0.3

def mm1_piece(i, t, hT, w1_ref, b1s, U):
    cols = pl.ds(pl.multiple_of(i * BF + t * 128, 128), 128)
    u = jnp.dot(upk(hT[...]), w1_ref[:, t * 128:(t + 1) * 128], preferred_element_type=f32) + b1s[:, cols]
    U[:, cols] = pk(gelu(u).astype(bf16))

def epilogue(j, y, xb, sT, o_ref):
    c0 = pl.multiple_of(j * BS, BS)
    o_ref[...] = (xb[:, pl.ds(c0, BS)].astype(f32) + upk(sT[:, pl.ds(c0, BS)]).astype(f32) * silu(y)).astype(bf16)

def kern(x_hbm, k_hbm, v_hbm, kk_hbm, sk_hbm, dv_hbm, w1_hbm, b1_hbm, w2_hbm, b2_hbm, fwd_hbm, inv_hbm,
         o_ref, hT, xnT, sT, U, par, pb, xb, kb, vb, kkb, w1b, w2b, b1s, b2s, ybuf,
         sk_ref, dv_ref, b1_ref, b2_ref, fwd_ref, inv_ref, sems):
    i = pl.program_id(0)
    slot = i % 2
    SW1, SK, SV, SKK, SW2, SX, SW10 = 0, 2, 4, 6, 8, 10, 10 + CH

    def x_copy(c): return pltpu.make_async_copy(x_hbm.at[:, c * CW:(c + 1) * CW], xb.at[:, c * CW:(c + 1) * CW], sems.at[SX + c])
    def w10_copy(c): return pltpu.make_async_copy(w1_hbm.at[c * CW:(c + 1) * CW, 0:BF], w1b.at[0, c * CW:(c + 1) * CW, :], sems.at[SW10 + c])
    def w1_copy(j, sl): return pltpu.make_async_copy(w1_hbm.at[:, pl.ds(pl.multiple_of(j * BF, 128), BF)], w1b.at[sl], sems.at[SW1 + sl])
    def grp_copies(j, sl):
        r = pl.ds(pl.multiple_of(j * GC, 16), GC)
        return [pltpu.make_async_copy(kk_hbm.at[r, :], kkb.at[sl], sems.at[SKK + sl]),
                pltpu.make_async_copy(k_hbm.at[r, :], kb.at[sl], sems.at[SK + sl]),
                pltpu.make_async_copy(v_hbm.at[r, :], vb.at[sl], sems.at[SV + sl])]
    def w2_copy(j, sl): return pltpu.make_async_copy(w2_hbm.at[:, pl.ds(pl.multiple_of(j * BS, BS), BS)], w2b.at[sl], sems.at[SW2 + sl])

    def run_order(order, g, gslot, mpiece):
        segA, segK, segQ, segP, segI = conv_segments(g, kb.at[gslot], vb.at[gslot], kkb.at[gslot], xnT, par, fwd_ref, inv_ref, sT, pb)
        for o in order:
            if o == 'A': segA()
            elif o == 'K': segK()
            elif o == 'I': segI()
            elif o[0] == 'Q': segQ(int(o[1:]))
            elif o[0] == 'P': segP(int(o[1:]))
            else: mpiece(int(o[1:]))

    def mm2_tile(j, sl):
        part = {}
        KH = F // 2
        c0 = pl.multiple_of(j * BS, BS)
        def mp(t):
            nt, kh = t // 2, t % 2
            part[t] = jnp.dot(upk(U[:, kh * KH:(kh + 1) * KH]), w2b[sl, kh * KH:(kh + 1) * KH, nt * 128:(nt + 1) * 128], preferred_element_type=f32)
            if kh == 1:
                ybuf[sl % YB, :, nt * 128:(nt + 1) * 128] = part[t - 1] + part[t] + b2s[:, pl.ds(pl.multiple_of(c0 + nt * 128, 128), 128)]
        return mp

    @pl.when(i == 0)
    def _():
      with jax.named_scope('s0'):
        seq = [('x', 0)]
        for c in range(CH):
            if c + 1 < CH: seq.append(('x', c + 1))
            seq.append(('w', c))
        nissued = [0]
        def issue_upto(n):
            while nissued[0] < min(n, len(seq)):
                kind, c = seq[nissued[0]]
                (x_copy(c) if kind == 'x' else w10_copy(c)).start()
                nissued[0] += 1
        issue_upto(min(PRE, PRE0))
        SS = 10 + 2 * CH
        smalls = [pltpu.make_async_copy(src, dst, sems.at[SS + n]) for n, (src, dst) in enumerate(
            [(sk_hbm, sk_ref), (dv_hbm, dv_ref), (b1_hbm, b1_ref), (b2_hbm, b2_ref), (fwd_hbm, fwd_ref), (inv_hbm, inv_ref)])]
        for cp in smalls: cp.start()
        issue_upto(PRE)
        def small_prep():
            par_prologue(sk_ref, dv_ref, par)
            b1s[...] = b1_ref[...].astype(f32).reshape(1, F)
            b2s[...] = b2_ref[...].astype(f32).reshape(1, S)
        if PARPOS < 0:
            for cp in smalls: cp.wait()
            small_prep()
        x_copy(0).wait()
        hs = {0: ln_chunk(xb, hT, xnT, 0)}
        acc = None
        for c in range(CH):
            if c + 1 < CH: x_copy(c + 1).wait()
            w10_copy(c).wait()
            if c == PARPOS:
                for cp in smalls: cp.wait()
            issue_upto(PRE + 2 * (c + 1))
            if c == max(CH - 1 - LATE, 0):
                issue_upto(len(seq))
                cps = grp_copies(0, 1)
                cps[0].start()
                if N1 > 1: w1_copy(1, 1).start()
                cps[1].start(); cps[2].start()
            d = jnp.dot(hs[c], w1b[0, c * CW:(c + 1) * CW, :], preferred_element_type=f32)
            acc = d if acc is None else acc + d
            if c == PARPOS: small_prep()
            if c + 1 < CH: hs[c + 1] = ln_chunk(xb, hT, xnT, c + 1)
        U[:, 0:BF] = pk(gelu(acc + b1s[:, 0:BF]).astype(bf16))

    @pl.when(jnp.logical_and(i >= 1, i < N1 - 1))
    def _():
        w1_copy(i + 1, 1 - slot).start()
    @pl.when(i == N1 - 1)
    def _():
        w2_copy(0, 0).start()
    @pl.when(jnp.logical_and(i >= 1, i < N1))
    def _():
      with jax.named_scope('ph1'):
        for cp in grp_copies(i, 1 - slot): cp.start()
        w1_copy(i, slot).wait()
        for cp in grp_copies(i - 1, slot): cp.wait()
        run_order(make_order(BF // 128), i - 1, slot, lambda t: mm1_piece(i, t, hT, w1b.at[slot], b1s, U))

    @pl.when(i == N1)
    def _():
      with jax.named_scope('ph1b'):
        if N2 > 1: w2_copy(1, 1).start()
        w2_copy(0, 0).wait()
        for cp in grp_copies(N1 - 1, N1 % 2): cp.wait()
        run_order(make_order(2 * (BS // 128)), N1 - 1, N1 % 2, mm2_tile(0, 0))

    @pl.when(jnp.logical_and(i > N1, i < N1 + N2 - 1))
    def _():
        w2_copy(i - N1 + 1, (i - N1 + 1) % 2).start()
    @pl.when(jnp.logical_and(i > N1, i < N1 + N2))
    def _():
      with jax.named_scope('ph2'):
        j = i - N1
        sl = j % 2
        w2_copy(j, sl).wait()
        ysl = sl if YB == 2 else 0
        ypr = 1 - sl if YB == 2 else 0
        epilogue(j - 1, ybuf[ypr], xb, sT, o_ref)
        if P2 == 1:
            ybuf[ysl] = jnp.dot(upk(U[...]), w2b[sl], preferred_element_type=f32) + b2s[:, pl.ds(pl.multiple_of(j * BS, BS), BS)]
        else:
            W = BS // P2
            for t in range(P2):
                ybuf[ysl, :, t * W:(t + 1) * W] = (jnp.dot(upk(U[...]), w2b[sl, :, t * W:(t + 1) * W], preferred_element_type=f32)
                                                  + b2s[:, pl.ds(pl.multiple_of(j * BS + t * W, W), W)])

    @pl.when(i == N1 + N2)
    def _():
      with jax.named_scope('fin'):
        epilogue(N2 - 1, ybuf[(N2 - 1) % 2 if YB == 2 else 0], xb, sT, o_ref)

@jax.jit
def pallas_recurrent_scan__ssm_conv_h3__mixer_token_mlp__prompt_kernel(A_q, A_k, A_v, A_shift_k, A_ssm_k, A_ssm_D, B_x, B_w1, B_b1, B_w2, B_b2):
    xT = A_q.reshape(S, D).T
    kT = A_k.reshape(S, D).T
    vT = A_v.reshape(S, D).T
    c2 = lambda i: (0, jnp.clip(i - N1 - 1, 0, N2 - 1))
    z = lambda i: (0, 0)
    z1 = lambda i: (0,)
    anyspec = pl.BlockSpec(memory_space=pl.ANY)
    u32 = jnp.uint32; bf = jnp.bfloat16
    outT = pl.pallas_call(kern,
        grid=(N1 + N2 + 1,),
        in_specs=[anyspec, anyspec, anyspec, anyspec,
                  anyspec, anyspec, anyspec, anyspec, anyspec, anyspec, anyspec, anyspec],
        out_specs=pl.BlockSpec((D, BS), c2),
        out_shape=jax.ShapeDtypeStruct((D, S), bf),
        scratch_shapes=[pltpu.VMEM((D // 2, S), u32), pltpu.VMEM((D // 2, S), u32),
                        pltpu.VMEM((D // 2, S), u32), pltpu.VMEM((D // 2, F), u32),
                        pltpu.VMEM((D, 5 * 128), f32), pltpu.VMEM((9 * NC * NT, 8, 128), f32),
                        pltpu.VMEM((D, S), bf), pltpu.VMEM((2, GC, S), bf), pltpu.VMEM((2, GC, S), bf), pltpu.VMEM((2, GC, S), bf),
                        pltpu.VMEM((2, S, BF), bf), pltpu.VMEM((2, F, BS), bf),
                        pltpu.VMEM((1, F), f32), pltpu.VMEM((1, S), f32), pltpu.VMEM((YB, D, BS), f32),
                        pltpu.VMEM((4, D), bf), pltpu.VMEM((D,), bf), pltpu.VMEM((F,), bf), pltpu.VMEM((S,), bf),
                        pltpu.VMEM((C, 2 * C), bf), pltpu.VMEM((2 * C, C), bf),
                        pltpu.SemaphoreType.DMA((10 + 2 * CH + 6,))],
        compiler_params=pltpu.CompilerParams(dimension_semantics=("arbitrary",), vmem_limit_bytes=110 << 20, disable_bounds_checks=bool(DBC)),
    )(xT, kT, vT, A_ssm_k, A_shift_k.T, A_ssm_D, B_w1, B_b1, B_w2, B_b2,
      jnp.asarray(_FWD), jnp.asarray(_INV))
    return outT.T.reshape(1, S, D)
```

```python
import jax
import jax.numpy as jnp
import numpy as np
from jax.experimental import pallas as pl
from jax.experimental.pallas import tpu as pltpu

S, D, F = 2048, 576, 4608
N1, N2 = 6, 8
BF, BS = F // N1, S // N2
GC = D // N1
NT = GC // 8
C = 128
NC = S // C
EPS = 1e-5
CWS = (128, 128, 256, 512, 512, 512)
CH = len(CWS)
CB = tuple(sum(CWS[:c]) for c in range(CH + 1))
PRE = 7
MB = 4

f32, bf16, u32 = jnp.float32, jnp.bfloat16, jnp.uint32


def _dft_mats():
    t = np.arange(C)[:, None]
    j = np.arange(C)[None, :]
    th = np.pi * (4 * j + 1) * t / (2 * C)
    fwd = np.concatenate([np.cos(th), np.sin(th)], axis=1)
    inv = fwd.T / C
    return fwd.astype(bf16), inv.astype(bf16)


_FWD, _INV = _dft_mats()


def _pk(a):
    return pltpu.bitcast(a, u32)


def _upk(a):
    return pltpu.bitcast(a, bf16)


def _gelu(u):
    c = 0.7978845608028654
    hu = 0.5 * u
    return hu + hu * jnp.tanh(u * (c + (c * 0.044715) * (u * u)))


def _silu(y):
    hy = 0.5 * y
    return hy + hy * jnp.tanh(hy)


def _stack(a):
    return jnp.concatenate([a[:, c * C:(c + 1) * C] for c in range(NC)], axis=0)


def _ln_chunk(xb, hT, xnT, c):
    cs = slice(CB[c], CB[c + 1])
    x = xb[:, cs].astype(f32)
    m = jnp.sum(x, axis=0, keepdims=True) * (1.0 / D)
    xc = x - m
    var = jnp.sum(xc * xc, axis=0, keepdims=True) * (1.0 / D)
    r1 = jax.lax.rsqrt(var + EPS)
    r2 = jax.lax.rsqrt(var * r1 * r1 + EPS)
    xnT[:, cs] = _pk((xc * r1).astype(bf16))
    h = (xc * (r1 * r2)).astype(bf16)
    hT[:, cs] = _pk(h)
    return h


def _conv_segments(g, k_ref, v_ref, kk_ref, xnT, par, fwd_ref, inv_ref, sT, pb):
    st = {}
    r0 = pl.multiple_of(g * GC, GC)

    def tap(j):
        t = par[pl.ds(r0, GC), j * 128:(j + 1) * 128]
        return jnp.concatenate([t] * NC, axis=1)

    def seg_a():
        kf = k_ref[...].astype(f32)
        lane = jax.lax.broadcasted_iota(jnp.int32, (GC, 128), 1)
        acc = None
        for j in range(4):
            if j == 0:
                kj = kf
            else:
                rj = pltpu.roll(kf, j, axis=1)
                kj = jnp.concatenate([jnp.where(lane >= j, rj[:, :128], 0.0), rj[:, 128:]], axis=1)
            acc = kj * tap(j) if acc is None else acc + kj * tap(j)
        kv = acc * v_ref[...].astype(f32)
        st['kv'] = kv
        st['X'] = jnp.dot(_stack(kv.astype(bf16)), fwd_ref[...], preferred_element_type=f32)

    def seg_k():
        st['K'] = jnp.dot(_stack(kk_ref[...]), fwd_ref[...], preferred_element_type=f32)

    names = ('a', 'b', 's', 'c', 'e', 'f', 'zre', 'zim')
    off = {n: k * NC * NT for k, n in enumerate(names)}
    zs = [pl.program_id(0) >> 6, pl.program_id(0) >> 7]
    cnt = [0]

    def nz():
        cnt[0] += 1
        return zs[cnt[0] % 2]

    def slot(n, i, r):
        return off[n] + i * NT + r

    def seg_q(r):
        X, K = st['X'], st['K']

        def t(A, i, part):
            return A[i * GC + r * 8:i * GC + r * 8 + 8, part * C:(part + 1) * C]

        for i in range(NC):
            a, b = t(X, i, 0), t(X, i, 1)
            pb[slot('a', i, r)] = a
            pb[slot('b', i, r)] = b
            pb[slot('s', i, r)] = a + b
        for d in range(NC):
            kre, kim = t(K, d, 0), t(K, d, 1)
            if d == 0:
                c, dd = kre, kim
            else:
                c, dd = kre + t(K, d - 1, 1), kim - t(K, d - 1, 0)
            pb[slot('c', d, r)] = c
            pb[slot('e', d, r)] = dd - c
            pb[slot('f', d, r)] = c + dd

    def rconv(p, q):
        out = []
        for m0 in range(0, NC, MB):
            ms = range(m0, min(m0 + MB, NC))
            k = {m: None for m in ms}
            for i in range(ms[-1] + 1):
                for m in ms:
                    if i <= m:
                        pr = q[m - i] * p[i]
                        k[m] = pr if k[m] is None else k[m] + pr
            out += [k[m] for m in ms]
        return out

    def seg_p(r):
        z = nz()
        k1 = rconv([pb[z + slot('s', i, r)] for i in range(NC)], [pb[z + slot('c', i, r)] for i in range(NC)])
        k3 = rconv([pb[z + slot('b', i, r)] for i in range(NC)], [pb[z + slot('f', i, r)] for i in range(NC)])
        for m in range(NC):
            pb[z + slot('zre', m, r)] = k1[m] - k3[m]
        z = nz()
        k2 = rconv([pb[z + slot('a', i, r)] for i in range(NC)], [pb[z + slot('e', i, r)] for i in range(NC)])
        for m in range(NC):
            pb[z + slot('zim', m, r)] = k1[m] + k2[m]

    def seg_i():
        z = nz()
        rows = []
        for m in range(NC):
            re = jnp.concatenate([pb[z + slot('zre', m, r)] for r in range(NT)], axis=0)
            im = jnp.concatenate([pb[z + slot('zim', m, r)] for r in range(NT)], axis=0)
            rows.append(jnp.concatenate([re, im], axis=1))
        Z = jnp.concatenate(rows, axis=0)
        Y = jnp.dot(Z.astype(bf16), inv_ref[...], preferred_element_type=f32)
        y = jnp.concatenate([Y[m * GC:(m + 1) * GC, :] for m in range(NC)], axis=1)
        r0h = pl.multiple_of(g * (GC // 2), GC // 2)
        sv = _upk(xnT[pl.ds(r0h, GC // 2), :]).astype(f32) * (y + st['kv'] * tap(4))
        sT[pl.ds(r0h, GC // 2), :] = _pk(sv.astype(bf16))

    return seg_a, seg_k, seg_q, seg_p, seg_i


def _order(npieces):
    order = ['K', 'M0', 'A'] + ['Q%d' % r for r in range(NT)]
    mid = list(range(1, npieces - 1))
    ev = [((r + 0.5) / NT, 'P%d' % r) for r in range(NT)]
    ev += [((k + 0.3) / max(len(mid), 1), 'M%d' % t) for k, t in enumerate(mid)]
    return order + [e[1] for e in sorted(ev)] + ['I', 'M%d' % (npieces - 1)]


def _kernel(x_hbm, k_hbm, v_hbm, kk_hbm, sk_hbm, dv_hbm, w1_hbm, b1_hbm, w2_hbm, b2_hbm, fwd_hbm, inv_hbm,
            o_ref, hT, xnT, sT, U, par, pb, xb, kb, vb, kkb, w1b, w2b, b1s, b2s, ybuf,
            sk_ref, dv_ref, b1_ref, b2_ref, fwd_ref, inv_ref, sems):
    i = pl.program_id(0)
    slot = i % 2
    SW1, SK, SV, SKK, SW2, SX, SW10, SS = 0, 2, 4, 6, 8, 10, 10 + CH, 10 + 2 * CH

    def x_copy(c):
        return pltpu.make_async_copy(x_hbm.at[:, CB[c]:CB[c + 1]], xb.at[:, CB[c]:CB[c + 1]], sems.at[SX + c])

    def w10_copy(c):
        return pltpu.make_async_copy(w1_hbm.at[CB[c]:CB[c + 1], 0:BF], w1b.at[0, CB[c]:CB[c + 1], :],
                                     sems.at[SW10 + c])

    def w1_copy(j, sl):
        return pltpu.make_async_copy(w1_hbm.at[:, pl.ds(pl.multiple_of(j * BF, 128), BF)], w1b.at[sl],
                                     sems.at[SW1 + sl])

    def grp_copies(j, sl):
        r = pl.ds(pl.multiple_of(j * GC, 16), GC)
        return [pltpu.make_async_copy(kk_hbm.at[r, :], kkb.at[sl], sems.at[SKK + sl]),
                pltpu.make_async_copy(k_hbm.at[r, :], kb.at[sl], sems.at[SK + sl]),
                pltpu.make_async_copy(v_hbm.at[r, :], vb.at[sl], sems.at[SV + sl])]

    def w2_copy(j, sl):
        return pltpu.make_async_copy(w2_hbm.at[:, pl.ds(pl.multiple_of(j * BS, BS), BS)], w2b.at[sl],
                                     sems.at[SW2 + sl])

    def run_group(g, gslot, npieces, mpiece):
        seg_a, seg_k, seg_q, seg_p, seg_i = _conv_segments(
            g, kb.at[gslot], vb.at[gslot], kkb.at[gslot], xnT, par, fwd_ref, inv_ref, sT, pb)
        for o in _order(npieces):
            if o == 'A':
                seg_a()
            elif o == 'K':
                seg_k()
            elif o == 'I':
                seg_i()
            elif o[0] == 'Q':
                seg_q(int(o[1:]))
            elif o[0] == 'P':
                seg_p(int(o[1:]))
            else:
                mpiece(int(o[1:]))

    def epilogue(j):
        cs = pl.ds(pl.multiple_of(j * BS, BS), BS)
        o_ref[...] = (xb[:, cs].astype(f32) + _upk(sT[:, cs]).astype(f32) * _silu(ybuf[...])).astype(bf16)

    @pl.when(i == 0)
    def _():
        seq = [x_copy(0)]
        for c in range(CH):
            if c + 1 < CH:
                seq.append(x_copy(c + 1))
            seq.append(w10_copy(c))
        issued = [0]

        def issue_upto(n):
            while issued[0] < min(n, len(seq)):
                seq[issued[0]].start()
                issued[0] += 1

        smalls = [pltpu.make_async_copy(src, dst, sems.at[SS + n]) for n, (src, dst) in enumerate(
            [(sk_hbm, sk_ref), (dv_hbm, dv_ref), (b1_hbm, b1_ref), (b2_hbm, b2_ref),
             (fwd_hbm, fwd_ref), (inv_hbm, inv_ref)])]
        for cp in smalls:
            cp.start()
        issue_upto(PRE)
        for cp in smalls:
            cp.wait()
        rows = jnp.concatenate([sk_ref[...].astype(f32), dv_ref[...].astype(f32).reshape(1, D),
                                jnp.zeros((3, D), f32)], axis=0)
        colT = rows.T
        for j in range(5):
            par[:, j * 128:(j + 1) * 128] = jnp.broadcast_to(colT[:, j:j + 1], (D, 128))
        b1s[...] = b1_ref[...].astype(f32).reshape(1, F)
        b2s[...] = b2_ref[...].astype(f32).reshape(1, S)
        x_copy(0).wait()
        hs = {0: _ln_chunk(xb, hT, xnT, 0)}
        acc = None
        for c in range(CH):
            if c + 1 < CH:
                x_copy(c + 1).wait()
            w10_copy(c).wait()
            issue_upto(PRE + 2 * (c + 1))
            if c == 0:
                issue_upto(len(seq))
                cps = grp_copies(0, 1)
                cps[0].start()
                w1_copy(1, 1).start()
                cps[1].start()
                cps[2].start()
            d = jnp.dot(hs[c], w1b[0, CB[c]:CB[c + 1], :], preferred_element_type=f32)
            acc = d if acc is None else acc + d
            if c + 1 < CH:
                hs[c + 1] = _ln_chunk(xb, hT, xnT, c + 1)
        U[:, 0:BF] = _pk(_gelu(acc + b1s[:, 0:BF]).astype(bf16))

    @pl.when(jnp.logical_and(i >= 1, i < N1 - 1))
    def _():
        w1_copy(i + 1, 1 - slot).start()

    @pl.when(i == N1 - 1)
    def _():
        w2_copy(0, 0).start()

    @pl.when(jnp.logical_and(i >= 1, i < N1))
    def _():
        for cp in grp_copies(i, 1 - slot):
            cp.start()
        w1_copy(i, slot).wait()
        for cp in grp_copies(i - 1, slot):
            cp.wait()

        def mm1_piece(t):
            cols = pl.ds(pl.multiple_of(i * BF + t * 128, 128), 128)
            u = jnp.dot(_upk(hT[...]), w1b[slot, :, t * 128:(t + 1) * 128], preferred_element_type=f32)
            U[:, cols] = _pk(_gelu(u + b1s[:, cols]).astype(bf16))

        run_group(i - 1, slot, BF // 128, mm1_piece)

    @pl.when(i == N1)
    def _():
        w2_copy(1, 1).start()
        w2_copy(0, 0).wait()
        for cp in grp_copies(N1 - 1, N1 % 2):
            cp.wait()
        part = {}
        KH = F // 2

        def mm2_piece(t):
            nt, kh = t // 2, t % 2
            part[t] = jnp.dot(_upk(U[:, kh * KH:(kh + 1) * KH]),
                              w2b[0, kh * KH:(kh + 1) * KH, nt * 128:(nt + 1) * 128],
                              preferred_element_type=f32)
            if kh == 1:
                ybuf[:, nt * 128:(nt + 1) * 128] = part[t - 1] + part[t] + b2s[:, nt * 128:(nt + 1) * 128]

        run_group(N1 - 1, N1 % 2, 2 * (BS // 128), mm2_piece)

    @pl.when(jnp.logical_and(i > N1, i < N1 + N2 - 1))
    def _():
        w2_copy(i - N1 + 1, (i - N1 + 1) % 2).start()

    @pl.when(jnp.logical_and(i > N1, i < N1 + N2))
    def _():
        j = i - N1
        sl = j % 2
        w2_copy(j, sl).wait()
        epilogue(j - 1)
        ybuf[...] = (jnp.dot(_upk(U[...]), w2b[sl], preferred_element_type=f32)
                     + b2s[:, pl.ds(pl.multiple_of(j * BS, BS), BS)])

    @pl.when(i == N1 + N2)
    def _():
        epilogue(N2 - 1)


@jax.jit
def pallas_recurrent_scan__ssm_conv_h3__mixer_token_mlp__prompt_kernel(
    A_q: jax.Array,
    A_k: jax.Array,
    A_v: jax.Array,
    A_shift_k: jax.Array,
    A_ssm_k: jax.Array,
    A_ssm_D: jax.Array,
    B_x: jax.Array,
    B_w1: jax.Array,
    B_b1: jax.Array,
    B_w2: jax.Array,
    B_b2: jax.Array,
):
    del B_x
    xT = A_q.reshape(S, D).T
    kT = A_k.reshape(S, D).T
    vT = A_v.reshape(S, D).T
    anyspec = pl.BlockSpec(memory_space=pl.ANY)
    outT = pl.pallas_call(
        _kernel,
        grid=(N1 + N2 + 1,),
        in_specs=[anyspec] * 12,
        out_specs=pl.BlockSpec((D, BS), lambda i: (0, jnp.clip(i - N1 - 1, 0, N2 - 1))),
        out_shape=jax.ShapeDtypeStruct((D, S), bf16),
        scratch_shapes=[
            pltpu.VMEM((D // 2, S), u32),
            pltpu.VMEM((D // 2, S), u32),
            pltpu.VMEM((D // 2, S), u32),
            pltpu.VMEM((D // 2, F), u32),
            pltpu.VMEM((D, 5 * 128), f32),
            pltpu.VMEM((8 * NC * NT, 8, 128), f32),
            pltpu.VMEM((D, S), bf16),
            pltpu.VMEM((2, GC, S), bf16),
            pltpu.VMEM((2, GC, S), bf16),
            pltpu.VMEM((2, GC, S), bf16),
            pltpu.VMEM((2, S, BF), bf16),
            pltpu.VMEM((2, F, BS), bf16),
            pltpu.VMEM((1, F), f32),
            pltpu.VMEM((1, S), f32),
            pltpu.VMEM((D, BS), f32),
            pltpu.VMEM((4, D), bf16),
            pltpu.VMEM((D,), bf16),
            pltpu.VMEM((F,), bf16),
            pltpu.VMEM((S,), bf16),
            pltpu.VMEM((C, 2 * C), bf16),
            pltpu.VMEM((2 * C, C), bf16),
            pltpu.SemaphoreType.DMA((10 + 2 * CH + 6,)),
        ],
        compiler_params=pltpu.CompilerParams(
            dimension_semantics=("arbitrary",),
            vmem_limit_bytes=110 << 20,
            disable_bounds_checks=True,
        ),
    )(xT, kT, vT, A_ssm_k, A_shift_k.T, A_ssm_D, B_w1, B_b1, B_w2, B_b2,
      jnp.asarray(_FWD), jnp.asarray(_INV))
    return outT.T.reshape(1, S, D)
```
